```python
import jax
import jax.numpy as jnp

def _softmax(x, axis=-1):
    return jax.nn.softmax(x, axis=axis)
def _gelu(x):
    return jax.nn.gelu(x, approximate=True)
def _silu(x):
    return jax.nn.silu(x)
def _sigmoid(x):
    return jax.nn.sigmoid(x)
def _layernorm(x, axis=-1, eps=1e-5):
    m = jnp.mean(x, axis=axis, keepdims=True)
    v = jnp.var(x, axis=axis, keepdims=True)
    return (x - m) / jnp.sqrt(v + eps)
def _scatter_add(tgt, idx, src, axis=0):
    return tgt.at[idx].add(src)
def _segment_sum(src, seg, n):
    return jax.ops.segment_sum(src, seg, n)
class _Rng:
    def __init__(self, key):
        self._k = key
    def _next(self):
        self._k, sub = jax.random.split(self._k)
        return sub
    def normal(self, shape):
        return jax.random.normal(self._next(), shape, dtype=jnp.bfloat16)
    def randint(self, lo, hi, shape):
        return jax.random.randint(self._next(), shape, lo, hi, dtype=jnp.int32)
    def uniform(self, shape, lo=0.0, hi=1.0):
        return jax.random.uniform(self._next(), shape, jnp.bfloat16, lo, hi)
    def permutation(self, n):
        return jax.random.permutation(self._next(), n)


kernel_name = 'recurrent_scan__sliding_block_cached__glu_gated_glu__decode'

def setup_inputs():
    _rng = _Rng(jax.random.key(int.from_bytes(__import__("os").urandom(4), "little")))
    _w = (lambda a: (lambda t: t.astype(jnp.bfloat16) if jnp.issubdtype(t.dtype, jnp.floating) else t)(jnp.asarray(a)))
    def _A_setup():
        B, Sq, D = 1, 1, 576
        Hq, Hkv, Sk, Dh = 32, 16, 65536, 128
        assert Hq % Hkv == 0, (Hq, Hkv)
        return {
            "x": _w((lambda *s: _rng.normal(s) * 0.05)(B, Sq, D)),
            "k_cache": _w((lambda *s: _rng.normal(s) * 0.05)(B, Hkv, Sk, Dh)),
            "v_cache": _w((lambda *s: _rng.normal(s) * 0.05)(B, Hkv, Sk, Dh)),
            "wq": _w((lambda *s: _rng.normal(s) * 0.05)(D, Hq * Dh) * (D ** -0.5)),
            "wo": _w((lambda *s: _rng.normal(s) * 0.05)(Hq * Dh, D) * ((Hq * Dh) ** -0.5)),
        }
    _A_in = _A_setup()

    def _B_setup():
        B, S, D, F = 1, 1, 576, 4608
        return {
            "x": _w((lambda *s: _rng.normal(s) * 0.05)(B, S, D)),
            "w_gate": _w((lambda *s: _rng.normal(s) * 0.05)(D, F)),
            "w_up": _w((lambda *s: _rng.normal(s) * 0.05)(D, F)),
            "w_down": _w((lambda *s: _rng.normal(s) * 0.05)(F, D)),
        }
    _B_in = _B_setup()

    return {
        "A_x": _A_in["x"],
        "A_k_cache": _A_in["k_cache"],
        "A_v_cache": _A_in["v_cache"],
        "A_wq": _A_in["wq"],
        "A_wo": _A_in["wo"],
        "B_x": _B_in["x"],
        "B_w_gate": _B_in["w_gate"],
        "B_w_up": _B_in["w_up"],
        "B_w_down": _B_in["w_down"],
    }

def reference(A_x, A_k_cache, A_v_cache, A_wq, A_wo, B_x, B_w_gate, B_w_up, B_w_down):
    def _A_ref(x, k_cache, v_cache, wq, wo):
        B, Sq, D = x.shape
        Hq, Dh = 32, 128
        Hkv, Sk = k_cache.shape[1], k_cache.shape[2]
        W = min(4096, max(256, Sk // 4))
        rep = Hq // Hkv
        q = (lambda x, *d: x.transpose(*d))((x @ wq).reshape(B, Sq, Hq, Dh), 0, 2, 1, 3)
        k = jnp.repeat(k_cache[:, :, Sk - W:, :], rep, axis=1)
        v = jnp.repeat(v_cache[:, :, Sk - W:, :], rep, axis=1)
        scores = jnp.einsum("bhqd,bhkd->bhqk", q, k) * (Dh ** -0.5)
        p = _softmax(scores, axis=-1)
        o = jnp.einsum("bhqk,bhkd->bhqd", p, v)
        return (lambda x, *d: x.transpose(*d))(o, 0, 2, 1, 3).reshape(B, Sq, Hq * Dh) @ wo

    def _B_ref(x, w_gate, w_up, w_down):
        g = jnp.einsum("bsd,df->bsf", x, w_gate)
        u = jnp.einsum("bsd,df->bsf", x, w_up)
        h = _sigmoid(g) * u
        return jnp.einsum("bsf,fd->bsd", h, w_down)

    x = A_x
    xn = _layernorm(x, axis=-1)
    s = _A_ref(xn, A_k_cache, A_v_cache, A_wq, A_wo)
    g = _silu(_B_ref(xn, B_w_gate, B_w_up, B_w_down))
    return x + s * g
```

```python
import jax
import jax.numpy as jnp
from jax import lax
import jax.experimental.pallas as pl
import jax.experimental.pallas.tpu as pltpu

_HQ, _DH = 32, 128
_M = 8
_NSEM = 4
_NT = (((1,), (1,)), ((), ()))


def _kernel(x_hbm, k_hbm, v_hbm, wq_hbm, wot_hbm, wg_hbm, wu_hbm, wdt_hbm, o_hbm,
            xb, kb, vb, wqb, wotb, wgb, wub, wdtb, qs, att, hid, ob, sems, iosem):
    f32, bf16 = jnp.float32, jnp.bfloat16
    hkv, sk = k_hbm.shape[1], k_hbm.shape[2]
    win = kb.shape[1]
    d_model = xb.shape[-1]
    d_ff = wgb.shape[1]
    ahead = _NSEM // 2

    def kcp(h):
        return pltpu.make_async_copy(
            k_hbm.at[0, h, pl.ds(sk - win, win), :], kb.at[h], sems.at[(2 * h + 1) % _NSEM])

    def vcp(h):
        return pltpu.make_async_copy(
            v_hbm.at[0, h, pl.ds(sk - win, win), :], vb.at[h], sems.at[(2 * h + 2) % _NSEM])

    wo_rows = [(r, min(128, d_model - r)) for r in range(0, d_model, 128)]
    tail = [(wg_hbm, wgb), (wu_hbm, wub), (wdt_hbm, wdtb)] + [
        (wot_hbm.at[pl.ds(r, n), :], wotb.at[pl.ds(r, n), :]) for r, n in wo_rows]
    first_tail = 2 * hkv + 1
    tcp = [pltpu.make_async_copy(s, d, sems.at[(first_tail + i) % _NSEM])
           for i, (s, d) in enumerate(tail)]

    def tail_wait(i):
        tcp[i].wait()
        if i + _NSEM < len(tcp):
            tcp[i + _NSEM].start()

    qcp = pltpu.make_async_copy(wq_hbm, wqb, sems.at[0])
    xcp = pltpu.make_async_copy(x_hbm, xb, iosem)
    xcp.start()
    qcp.start()
    for i in range(1, _NSEM):
        (kcp(i // 2) if i % 2 else vcp(i // 2 - 1)).start()

    xcp.wait()
    x = xb[0].astype(f32)
    xc = x - jnp.mean(x, axis=-1, keepdims=True)
    xn = xc / jnp.sqrt(jnp.mean(xc * xc, axis=-1, keepdims=True) + 1e-5)
    xn = jnp.broadcast_to(xn, (_M, d_model)).astype(bf16)

    row = lax.broadcasted_iota(jnp.int32, (_M, _DH), 0)
    qcp.wait()
    vcp(ahead - 1).start()
    qc = 512

    def q_body(c, carry):
        q = jnp.dot(xn, wqb[:, pl.ds(pl.multiple_of(c * qc, qc), qc)],
                    preferred_element_type=f32)
        for j in range(qc // (2 * _DH)):
            qs[c * (qc // (2 * _DH)) + j] = jnp.where(
                row == 0, q[:, 2 * j * _DH:(2 * j + 1) * _DH],
                q[:, (2 * j + 1) * _DH:(2 * j + 2) * _DH])
        return carry

    lax.fori_loop(0, _HQ * _DH // qc, q_body, 0)

    def head_body(h, carry):
        kcp(h).wait()

        @pl.when(h + ahead < hkv)
        def _():
            kcp(h + ahead).start()

        for t in range(ahead):
            @pl.when(h + ahead == hkv + t)
            def _():
                tcp[2 * t].start()

        s = lax.dot_general(qs[h].astype(bf16), kb[h], _NT,
                            preferred_element_type=f32) * (_DH ** -0.5)
        p = jnp.exp(s - jnp.max(s, axis=-1, keepdims=True))
        denom = jnp.sum(p, axis=-1, keepdims=True)

        vcp(h).wait()

        @pl.when(h + ahead < hkv)
        def _():
            vcp(h + ahead).start()

        for t in range(ahead):
            @pl.when(h + ahead == hkv + t)
            def _():
                tcp[2 * t + 1].start()

        o = jnp.dot(p.astype(bf16), vb[h], preferred_element_type=f32) / denom
        c0 = pl.multiple_of(h * 2 * _DH, 2 * _DH)
        att[:, pl.ds(c0, _DH)] = jnp.where(row == 0, o, 0.0)
        att[:, pl.ds(c0 + _DH, _DH)] = jnp.where(row == 1, o, 0.0)
        return carry

    lax.fori_loop(0, hkv, head_body, 0)

    fc = 512
    tail_wait(0)
    tail_wait(1)

    def glu_body(c, carry):
        c0 = pl.multiple_of(c * fc, fc)
        g = jnp.dot(xn, wgb[:, pl.ds(c0, fc)], preferred_element_type=f32)
        u = jnp.dot(xn, wub[:, pl.ds(c0, fc)], preferred_element_type=f32)
        hid[:, pl.ds(c0, fc)] = jax.nn.sigmoid(g) * u
        return carry

    lax.fori_loop(0, d_ff // fc, glu_body, 0)
    tail_wait(2)

    def down_body(c, acc):
        c0 = pl.multiple_of(c * fc, fc)
        return acc + lax.dot_general(hid[:, pl.ds(c0, fc)].astype(bf16), wdtb[:, pl.ds(c0, fc)],
                                     _NT, preferred_element_type=f32)

    y = lax.fori_loop(0, d_ff // fc, down_body, jnp.zeros((_M, d_model), f32))[0:1]
    gate = y * jax.nn.sigmoid(y)

    parts = []
    for i, (r, n) in enumerate(wo_rows):
        tail_wait(3 + i)
        pr = lax.dot_general(att[...].astype(bf16), wotb[r:r + n, :], _NT,
                             preferred_element_type=f32)
        parts.append(jnp.sum(pr, axis=0, keepdims=True))
    ob[0] = (x + jnp.concatenate(parts, axis=1) * gate).astype(bf16)
    ocp = pltpu.make_async_copy(ob, o_hbm, iosem)
    ocp.start()
    ocp.wait()


@jax.jit
def pallas_recurrent_scan__sliding_block_cached__glu_gated_glu__decode_kernel(
    A_x: jax.Array,
    A_k_cache: jax.Array,
    A_v_cache: jax.Array,
    A_wq: jax.Array,
    A_wo: jax.Array,
    B_x: jax.Array,
    B_w_gate: jax.Array,
    B_w_up: jax.Array,
    B_w_down: jax.Array,
):
    del B_x
    d_model = A_x.shape[-1]
    hkv, sk = A_k_cache.shape[1:3]
    d_ff = B_w_gate.shape[1]
    win = min(4096, max(256, sk // 4))
    assert A_x.shape[:2] == (1, 1) and _HQ == 2 * hkv
    bf16, f32 = jnp.bfloat16, jnp.float32
    hbm = pl.BlockSpec(memory_space=pltpu.HBM)
    return pl.pallas_call(
        _kernel,
        out_shape=jax.ShapeDtypeStruct(A_x.shape, bf16),
        in_specs=[hbm] * 8,
        out_specs=hbm,
        scratch_shapes=[
            pltpu.VMEM(A_x.shape, bf16),
            pltpu.VMEM((hkv, win, _DH), bf16),
            pltpu.VMEM((hkv, win, _DH), bf16),
            pltpu.VMEM((d_model, _HQ * _DH), bf16),
            pltpu.VMEM((d_model, _HQ * _DH), bf16),
            pltpu.VMEM((d_model, d_ff), bf16),
            pltpu.VMEM((d_model, d_ff), bf16),
            pltpu.VMEM((d_model, d_ff), bf16),
            pltpu.VMEM((hkv, _M, _DH), f32),
            pltpu.VMEM((_M, _HQ * _DH), f32),
            pltpu.VMEM((_M, d_ff), f32),
            pltpu.VMEM(A_x.shape, bf16),
            pltpu.SemaphoreType.DMA((_NSEM,)),
            pltpu.SemaphoreType.DMA(()),
        ],
        compiler_params=pltpu.CompilerParams(vmem_limit_bytes=100 * 2**20),
    )(A_x, A_k_cache, A_v_cache, A_wq, A_wo.T, B_w_gate, B_w_up, B_w_down.T)
```

```python
import jax
import jax.numpy as jnp
from jax import lax
import jax.experimental.pallas as pl
import jax.experimental.pallas.tpu as pltpu

_HQ, _DH = 32, 128
_M = 8
_NSEM = 4
_NT = (((1,), (1,)), ((), ()))


def _kernel(x_hbm, k_hbm, v_hbm, wq_hbm, wot_hbm, wg_hbm, wu_hbm, wdt_hbm, o_hbm,
            xb, kb, vb, wqb, wotb, wgb, wub, wdtb, qs, att, hid, ob, sems):
    f32, bf16 = jnp.float32, jnp.bfloat16
    hkv, sk = k_hbm.shape[1], k_hbm.shape[2]
    win = kb.shape[1]
    d_model = xb.shape[-1]
    d_attn = wotb.shape[1]
    d_ff = wgb.shape[1]

    blocks = [(r, min(128, d_model - r)) for r in range(0, d_model, 128)]
    blocks = blocks[-1:] + blocks[:-1]
    e = d_attn // 8
    wo_pieces = [(r, n, 0, d_attn) for r, n in blocks[:-1]] + [
        (*blocks[-1], c * e, w * e) for c, w in ((0, 4), (4, 2), (6, 1), (7, 1))]

    def kcp(h):
        return pltpu.make_async_copy(
            k_hbm.at[0, h, pl.ds(sk - win, win), :], kb.at[h], sems.at[(2 * h + 2) % _NSEM])

    def vcp(h):
        return pltpu.make_async_copy(
            v_hbm.at[0, h, pl.ds(sk - win, win), :], vb.at[h], sems.at[(2 * h + 3) % _NSEM])

    first_tail = 2 * hkv + 2
    tail = [(wg_hbm, wgb), (wu_hbm, wub), (wdt_hbm, wdtb)] + [
        (wot_hbm.at[pl.ds(r, n), pl.ds(c, w)], wotb.at[pl.ds(r, n), pl.ds(c, w)])
        for r, n, c, w in wo_pieces]
    tcp = [pltpu.make_async_copy(s, d, sems.at[(first_tail + i) % _NSEM])
           for i, (s, d) in enumerate(tail)]
    qcp = pltpu.make_async_copy(wq_hbm, wqb, sems.at[0])
    xcp = pltpu.make_async_copy(x_hbm, xb, sems.at[1])
    ocp = pltpu.make_async_copy(ob, o_hbm, sems.at[(first_tail + len(tail)) % _NSEM])

    def start_kv(i):
        (vcp if i % 2 else kcp)(i // 2).start()

    def start_after_kv(h, is_v):
        j = is_v + _NSEM

        @pl.when(h + j // 2 < hkv)
        def _():
            (vcp if j % 2 else kcp)(h + j // 2).start()

        for last in range(hkv - j // 2, hkv):
            @pl.when(h == last)
            def _():
                tcp[2 * (last - hkv) + j].start()

    def tail_wait(i):
        tcp[i].wait()
        if i + _NSEM < len(tcp):
            tcp[i + _NSEM].start()

    qcp.start()
    xcp.start()
    for i in range(_NSEM - 2):
        start_kv(i)
    qcp.wait()
    start_kv(_NSEM - 2)
    xcp.wait()
    start_kv(_NSEM - 1)

    x = xb[0].astype(f32)
    xc = x - jnp.mean(x, axis=-1, keepdims=True)
    xn = xc / jnp.sqrt(jnp.mean(xc * xc, axis=-1, keepdims=True) + 1e-5)
    xn = jnp.broadcast_to(xn, (_M, d_model)).astype(bf16)

    row = lax.broadcasted_iota(jnp.int32, (_M, _DH), 0)
    qc = 512

    def q_body(c, carry):
        q = jnp.dot(xn, wqb[:, pl.ds(pl.multiple_of(c * qc, qc), qc)],
                    preferred_element_type=f32)
        for j in range(qc // (2 * _DH)):
            qs[c * (qc // (2 * _DH)) + j] = jnp.where(
                row == 0, q[:, 2 * j * _DH:(2 * j + 1) * _DH],
                q[:, (2 * j + 1) * _DH:(2 * j + 2) * _DH])
        return carry

    lax.fori_loop(0, d_attn // qc, q_body, 0)

    def head_body(h, carry):
        kcp(h).wait()
        start_after_kv(h, 0)
        s = lax.dot_general(qs[h].astype(bf16), kb[h], _NT,
                            preferred_element_type=f32) * (_DH ** -0.5)
        p = jnp.exp(s - jnp.max(s, axis=-1, keepdims=True))
        denom = jnp.sum(p, axis=-1, keepdims=True)
        vcp(h).wait()
        start_after_kv(h, 1)
        o = jnp.dot(p.astype(bf16), vb[h], preferred_element_type=f32) / denom
        c0 = pl.multiple_of(h * 2 * _DH, 2 * _DH)
        att[:, pl.ds(c0, _DH)] = jnp.broadcast_to(o[0:1], (_M, _DH))
        att[:, pl.ds(c0 + _DH, _DH)] = jnp.broadcast_to(o[1:2], (_M, _DH))
        return carry

    lax.fori_loop(0, hkv, head_body, 0)

    fc = 512
    tail_wait(0)
    tail_wait(1)

    def glu_body(c, carry):
        c0 = pl.multiple_of(c * fc, fc)
        g = jnp.dot(xn, wgb[:, pl.ds(c0, fc)], preferred_element_type=f32)
        u = jnp.dot(xn, wub[:, pl.ds(c0, fc)], preferred_element_type=f32)
        hid[:, pl.ds(c0, fc)] = jax.nn.sigmoid(g) * u
        return carry

    lax.fori_loop(0, d_ff // fc, glu_body, 0)
    tail_wait(2)

    def down_body(c, acc):
        c0 = pl.multiple_of(c * fc, fc)
        return acc + lax.dot_general(hid[:, pl.ds(c0, fc)].astype(bf16), wdtb[:, pl.ds(c0, fc)],
                                     _NT, preferred_element_type=f32)

    y = lax.fori_loop(0, d_ff // fc, down_body, jnp.zeros((_M, d_model), f32))[0:1]
    gate = y * jax.nn.sigmoid(y)

    acc = None
    for i, (r, n, c, w) in enumerate(wo_pieces):
        lhs = att[:, c:c + w].astype(bf16)
        tail_wait(3 + i)
        part = lax.dot_general(lhs, wotb[r:r + n, c:c + w], _NT,
                               preferred_element_type=f32)[0:1]
        acc = part if c == 0 else acc + part
        if c + w == d_attn:
            ob[0, :, r:r + n] = (x[:, r:r + n] + acc * gate[:, r:r + n]).astype(bf16)
    ocp.start()
    ocp.wait()


@jax.jit
def pallas_recurrent_scan__sliding_block_cached__glu_gated_glu__decode_kernel(
    A_x: jax.Array,
    A_k_cache: jax.Array,
    A_v_cache: jax.Array,
    A_wq: jax.Array,
    A_wo: jax.Array,
    B_x: jax.Array,
    B_w_gate: jax.Array,
    B_w_up: jax.Array,
    B_w_down: jax.Array,
):
    del B_x
    d_model = A_x.shape[-1]
    hkv, sk = A_k_cache.shape[1:3]
    d_ff = B_w_gate.shape[1]
    win = min(4096, max(256, sk // 4))
    assert A_x.shape[:2] == (1, 1) and _HQ == 2 * hkv
    bf16, f32 = jnp.bfloat16, jnp.float32
    hbm = pl.BlockSpec(memory_space=pltpu.HBM)
    return pl.pallas_call(
        _kernel,
        out_shape=jax.ShapeDtypeStruct(A_x.shape, bf16),
        in_specs=[hbm] * 8,
        out_specs=hbm,
        scratch_shapes=[
            pltpu.VMEM(A_x.shape, bf16),
            pltpu.VMEM((hkv, win, _DH), bf16),
            pltpu.VMEM((hkv, win, _DH), bf16),
            pltpu.VMEM((d_model, _HQ * _DH), bf16),
            pltpu.VMEM((d_model, _HQ * _DH), bf16),
            pltpu.VMEM((d_model, d_ff), bf16),
            pltpu.VMEM((d_model, d_ff), bf16),
            pltpu.VMEM((d_model, d_ff), bf16),
            pltpu.VMEM((hkv, _M, _DH), f32),
            pltpu.VMEM((_M, _HQ * _DH), f32),
            pltpu.VMEM((_M, d_ff), f32),
            pltpu.VMEM(A_x.shape, bf16),
            pltpu.SemaphoreType.DMA((_NSEM,)),
        ],
        compiler_params=pltpu.CompilerParams(vmem_limit_bytes=100 * 2**20),
    )(A_x, A_k_cache, A_v_cache, A_wq, A_wo.T, B_w_gate, B_w_up, B_w_down.T)
```
